```python
import os as _os
_os.environ.setdefault("JAX_PLATFORMS", "cpu")
import jax
import jax.numpy as jnp

def _softmax(x, axis=-1):
    return jax.nn.softmax(x, axis=axis)
def _gelu(x):
    return jax.nn.gelu(x, approximate=True)
def _silu(x):
    return jax.nn.silu(x)
def _sigmoid(x):
    return jax.nn.sigmoid(x)
def _layernorm(x, axis=-1, eps=1e-5):
    m = jnp.mean(x, axis=axis, keepdims=True)
    v = jnp.var(x, axis=axis, keepdims=True)
    return (x - m) / jnp.sqrt(v + eps)
def _scatter_add(tgt, idx, src, axis=0):
    return tgt.at[idx].add(src)
def _segment_sum(src, seg, n):
    return jax.ops.segment_sum(src, seg, n)
class _Rng:
    def __init__(self, key):
        self._k = key
    def _next(self):
        self._k, sub = jax.random.split(self._k)
        return sub
    def normal(self, shape):
        return jax.random.normal(self._next(), shape, dtype=jnp.bfloat16)
    def randint(self, lo, hi, shape):
        return jax.random.randint(self._next(), shape, lo, hi, dtype=jnp.int32)
    def uniform(self, shape, lo=0.0, hi=1.0):
        return jax.random.uniform(self._next(), shape, jnp.bfloat16, lo, hi)
    def permutation(self, n):
        return jax.random.permutation(self._next(), n)


kernel_name = 'standalone__mha_softmax__sampling'

def setup_inputs():
    _rng = _Rng(jax.random.key(int.from_bytes(__import__("os").urandom(4), "little")))
    _w = (lambda a: (lambda t: t.astype(jnp.bfloat16) if jnp.issubdtype(t.dtype, jnp.floating) else t)(jnp.asarray(a)))
    B, H, Sq, Sk, D = 8, 32, 32, 2048, 128
    return {
        "q": _w((lambda *s: _rng.normal(s) * 0.4)(B, H, Sq, D)),
        "k": _w((lambda *s: _rng.normal(s) * 0.4)(B, H, Sk, D)),
        "v": _w((lambda *s: _rng.normal(s) * 0.05)(B, H, Sk, D)),
    }

def reference(q, k, v):
    scale = q.shape[-1] ** -0.5
    scores = jnp.einsum("bhqd,bhkd->bhqk", q, k) * scale
    p = _softmax(scores, axis=-1)
    return jnp.einsum("bhqk,bhkd->bhqd", p, v)
```

```python
import math

import jax
import jax.numpy as jnp
import jax.experimental.pallas as pl
import jax.experimental.pallas.tpu as pltpu

_LANES = 128
_HEADS = 8
_STRIDE = 2
_KEYS = 256
_COPY_ROWS = 16
_SLOTS = 4
_MAX_INIT = -3.0e38


def _attention_kernel(q_hbm, k_hbm, v_hbm, o_hbm,
                      q_buf, k_buf, v_buf, o_buf, m_ref, l_ref, acc_ref,
                      q_sem, k_sem, v_sem, o_sem):
    n_super, heads, stride, _, d = q_hbm.shape
    n_groups = n_super * stride
    steps_per_group = k_hbm.shape[3] // _KEYS
    n_steps = n_groups * steps_per_group
    exp2_scale = (d ** -0.5) * math.log2(math.e)

    def fetch(step):
        group, chunk, slot = step // steps_per_group, step % steps_per_group, step % _SLOTS
        for row in range(0, _KEYS, _COPY_ROWS):
            for queue, (src, dst, sem) in enumerate(
                    ((k_hbm, k_buf, k_sem), (v_hbm, v_buf, v_sem))):
                pltpu.make_async_copy(
                    src.at[group // stride, :, group % stride,
                           pl.ds(chunk * _KEYS + row, _COPY_ROWS)],
                    dst.at[slot, :, pl.ds(row, _COPY_ROWS)],
                    sem.at[slot]).start(priority=queue)

    def q_copy(sup):
        return pltpu.make_async_copy(q_hbm.at[sup], q_buf.at[sup], q_sem.at[sup % 2])

    def o_copy(*index):
        return pltpu.make_async_copy(o_buf.at[index], o_hbm.at[index], o_sem.at[0])

    def scores(group, slot, h):
        return jax.lax.dot_general(
            q_buf[group // stride, h, group % stride], k_buf[slot, h],
            (((1,), (1,)), ((), ())), preferred_element_type=jnp.float32)

    def accumulate(slot, h, s):
        tiles = [s[:, j:j + _LANES] for j in range(0, _KEYS, _LANES)]
        tile_max = tiles[0]
        for tile in tiles[1:]:
            tile_max = jnp.maximum(tile_max, tile)
        m_old = m_ref[h]
        m_new = jnp.maximum(m_old, jnp.max(tile_max, axis=-1, keepdims=True))
        alpha = jnp.exp2((m_old - m_new) * exp2_scale)
        probs = [jnp.exp2((tile - m_new) * exp2_scale) for tile in tiles]
        lane_sum = probs[0]
        for p in probs[1:]:
            lane_sum = lane_sum + p
        p = jnp.concatenate([p.astype(v_buf.dtype) for p in probs], axis=1)
        pv = jnp.dot(p, v_buf[slot, h], preferred_element_type=jnp.float32)
        m_ref[h] = m_new
        l_ref[h] = alpha * l_ref[h] + lane_sum
        acc_ref[h] = alpha * acc_ref[h] + pv

    def run_group(group, _):
        m_ref[...] = jnp.full(m_ref.shape, _MAX_INIT, jnp.float32)
        l_ref[...] = jnp.zeros(l_ref.shape, jnp.float32)
        acc_ref[...] = jnp.zeros(acc_ref.shape, jnp.float32)

        @pl.when(group % stride == 0)
        def _():
            q_copy(group // stride).wait()

            @pl.when(group // stride + 1 < n_super)
            def _():
                q_copy(group // stride + 1).start()

        def run_step(chunk, _):
            step = group * steps_per_group + chunk
            slot = step % _SLOTS
            pltpu.make_async_copy(k_buf.at[slot], k_buf.at[slot], k_sem.at[slot]).wait()
            pltpu.make_async_copy(v_buf.at[slot], v_buf.at[slot], v_sem.at[slot]).wait()

            @pl.when(step + _SLOTS - 1 < n_steps)
            def _():
                fetch(step + _SLOTS - 1)

            @pl.when(step == n_steps - 2)
            def _():
                half = (n_super - 1) // 2
                o_copy(pl.ds(0, half)).start(priority=0)
                o_copy(pl.ds(half, n_super - 1 - half)).start(priority=1)
                for p in range(stride - 1):
                    o_copy(n_super - 1, slice(None), p).start()

            all_scores = [scores(group, slot, h) for h in range(heads)]
            for h in range(heads):
                accumulate(slot, h, all_scores[h])

        jax.lax.fori_loop(0, steps_per_group, run_step, None)
        for h in range(heads):
            total = jnp.sum(l_ref[h], axis=-1, keepdims=True)
            o_buf[group // stride, h, group % stride] = (acc_ref[h] / total).astype(o_buf.dtype)

    q_copy(0).start()
    for step in range(_SLOTS - 1):
        fetch(step)
    jax.lax.fori_loop(0, n_groups, run_group, None)
    o_copy(n_super - 1, slice(None), stride - 1).start()
    pltpu.make_async_copy(o_buf, o_buf, o_sem.at[0]).wait()


@jax.jit
def pallas_standalone__mha_softmax__sampling_kernel(
    q: jax.Array,
    k: jax.Array,
    v: jax.Array,
):
    batch, n_heads, sq, d = q.shape
    n_super = batch * n_heads // (_HEADS * _STRIDE)
    assert n_super * _HEADS * _STRIDE == batch * n_heads and n_super >= 3
    assert k.shape[2] % _KEYS == 0 and k.shape[2] >= 2 * _KEYS and d == _LANES

    def grouped(x):
        return x.reshape(n_super, _HEADS, _STRIDE, x.shape[2], d)

    q_shape = (n_super, _HEADS, _STRIDE, sq, d)
    out = pl.pallas_call(
        _attention_kernel,
        in_specs=[pl.BlockSpec(memory_space=pl.ANY)] * 3,
        out_specs=pl.BlockSpec(memory_space=pl.ANY),
        out_shape=jax.ShapeDtypeStruct(q_shape, q.dtype),
        scratch_shapes=[
            pltpu.VMEM(q_shape, q.dtype),
            pltpu.VMEM((_SLOTS, _HEADS, _KEYS, d), k.dtype),
            pltpu.VMEM((_SLOTS, _HEADS, _KEYS, d), v.dtype),
            pltpu.VMEM(q_shape, q.dtype),
            pltpu.VMEM((_HEADS, sq, _LANES), jnp.float32),
            pltpu.VMEM((_HEADS, sq, _LANES), jnp.float32),
            pltpu.VMEM((_HEADS, sq, d), jnp.float32),
            pltpu.SemaphoreType.DMA((2,)),
            pltpu.SemaphoreType.DMA((_SLOTS,)),
            pltpu.SemaphoreType.DMA((_SLOTS,)),
            pltpu.SemaphoreType.DMA((1,)),
        ],
        compiler_params=pltpu.CompilerParams(vmem_limit_bytes=32 * 2**20),
    )(grouped(q), grouped(k), grouped(v))
    return out.reshape(q.shape)
```

```python
import math

import jax
import jax.numpy as jnp
import numpy as np
import jax.experimental.pallas as pl
import jax.experimental.pallas.tpu as pltpu

_LANES = 128
_HEADS = 8
_STRIDE = 2
_KEYS = 256
_COPY_HEADS = 2
_COPY_KEYS = 64
_SLOTS = 4
_LOWEST = float(np.finfo(np.float32).min)


def _attention_kernel(q_hbm, k_hbm, v_hbm, o_hbm,
                      q_buf, k_buf, v_buf, o_buf, m_ref, l_ref, acc_ref,
                      q_sem, k_sem, v_sem, o_sem):
    n_blocks, heads, stride, _, d = q_hbm.shape
    n_groups = n_blocks * stride
    steps_per_group = k_hbm.shape[3] // _KEYS
    n_steps = n_groups * steps_per_group
    exp2_scale = (d ** -0.5) * math.log2(math.e)

    def start_fetch(step):
        group, chunk, slot = step // steps_per_group, step % steps_per_group, step % _SLOTS
        for key in range(0, _KEYS, _COPY_KEYS):
            for head in range(0, heads, _COPY_HEADS):
                for src, dst, sem, queue in ((k_hbm, k_buf, k_sem, 1), (v_hbm, v_buf, v_sem, 0)):
                    pltpu.make_async_copy(
                        src.at[group // stride, pl.ds(head, _COPY_HEADS), group % stride,
                               pl.ds(chunk * _KEYS + key, _COPY_KEYS)],
                        dst.at[slot, pl.ds(head, _COPY_HEADS), pl.ds(key, _COPY_KEYS)],
                        sem.at[slot]).start(priority=queue)

    def wait_fetch(slot):
        pltpu.make_async_copy(k_buf.at[slot], k_buf.at[slot], k_sem.at[slot]).wait()
        pltpu.make_async_copy(v_buf.at[slot], v_buf.at[slot], v_sem.at[slot]).wait()

    q_copy = pltpu.make_async_copy(q_hbm, q_buf, q_sem)
    early_blocks, last_block = pl.ds(0, n_blocks - 1), n_blocks - 1
    early_o_copies = [
        pltpu.make_async_copy(o_buf.at[early_blocks, h], o_hbm.at[early_blocks, h], o_sem)
        for h in range(heads)]
    last_o_copy = pltpu.make_async_copy(o_buf.at[last_block], o_hbm.at[last_block], o_sem)

    def scores(group, slot, h):
        return jax.lax.dot_general(
            q_buf[group // stride, h, group % stride], k_buf[slot, h],
            (((1,), (1,)), ((), ())), preferred_element_type=jnp.float32)

    def accumulate(slot, h, s):
        tiles = [s[:, j:j + _LANES] for j in range(0, _KEYS, _LANES)]
        tile_max = tiles[0]
        for tile in tiles[1:]:
            tile_max = jnp.maximum(tile_max, tile)
        m_old = m_ref[h]
        m_new = jnp.maximum(m_old, jnp.max(tile_max, axis=-1, keepdims=True))
        alpha = jnp.exp2((m_old - m_new) * exp2_scale)
        probs = [jnp.exp2((tile - m_new) * exp2_scale) for tile in tiles]
        lane_sum = probs[0]
        for p in probs[1:]:
            lane_sum = lane_sum + p
        p = jnp.concatenate([p.astype(v_buf.dtype) for p in probs], axis=1)
        pv = jnp.dot(p, v_buf[slot, h], preferred_element_type=jnp.float32)
        m_ref[h] = m_new
        l_ref[h] = alpha * l_ref[h] + lane_sum
        acc_ref[h] = alpha * acc_ref[h] + pv

    def run_group(group, _):
        m_ref[...] = jnp.full(m_ref.shape, _LOWEST, jnp.float32)
        l_ref[...] = jnp.zeros(l_ref.shape, jnp.float32)
        acc_ref[...] = jnp.zeros(acc_ref.shape, jnp.float32)

        def run_step(chunk, _):
            step = group * steps_per_group + chunk
            slot = step % _SLOTS

            @pl.when(step + _SLOTS - 1 < n_steps)
            def _():
                start_fetch(step + _SLOTS - 1)

            wait_fetch(slot)

            @pl.when(step == n_steps - 2)
            def _():
                for copy in early_o_copies:
                    copy.start()

            all_scores = [scores(group, slot, h) for h in range(heads)]
            for h in range(heads):
                accumulate(slot, h, all_scores[h])

        jax.lax.fori_loop(0, steps_per_group, run_step, None)
        for h in range(heads):
            total = jnp.sum(l_ref[h], axis=-1, keepdims=True)
            o_buf[group // stride, h, group % stride] = (acc_ref[h] / total).astype(o_buf.dtype)

    q_copy.start()
    for step in range(_SLOTS - 1):
        start_fetch(step)
    q_copy.wait()
    jax.lax.fori_loop(0, n_groups, run_group, None)
    last_o_copy.start()
    for copy in early_o_copies + [last_o_copy]:
        copy.wait()


@jax.jit
def pallas_standalone__mha_softmax__sampling_kernel(
    q: jax.Array,
    k: jax.Array,
    v: jax.Array,
):
    batch, n_heads, n_queries, d = q.shape
    n_blocks = batch * n_heads // (_HEADS * _STRIDE)
    assert n_blocks * _HEADS * _STRIDE == batch * n_heads and n_blocks >= 2
    assert k.shape[2] % _KEYS == 0 and d == _LANES

    def blocked(x):
        return x.reshape(n_blocks, _HEADS, _STRIDE, x.shape[2], d)

    q_shape = (n_blocks, _HEADS, _STRIDE, n_queries, d)
    out = pl.pallas_call(
        _attention_kernel,
        in_specs=[pl.BlockSpec(memory_space=pl.ANY)] * 3,
        out_specs=pl.BlockSpec(memory_space=pl.ANY),
        out_shape=jax.ShapeDtypeStruct(q_shape, q.dtype),
        scratch_shapes=[
            pltpu.VMEM(q_shape, q.dtype),
            pltpu.VMEM((_SLOTS, _HEADS, _KEYS, d), k.dtype),
            pltpu.VMEM((_SLOTS, _HEADS, _KEYS, d), v.dtype),
            pltpu.VMEM(q_shape, q.dtype),
            pltpu.VMEM((_HEADS, n_queries, _LANES), jnp.float32),
            pltpu.VMEM((_HEADS, n_queries, _LANES), jnp.float32),
            pltpu.VMEM((_HEADS, n_queries, d), jnp.float32),
            pltpu.SemaphoreType.DMA,
            pltpu.SemaphoreType.DMA((_SLOTS,)),
            pltpu.SemaphoreType.DMA((_SLOTS,)),
            pltpu.SemaphoreType.DMA,
        ],
        compiler_params=pltpu.CompilerParams(vmem_limit_bytes=32 * 2**20),
    )(blocked(q), blocked(k), blocked(v))
    return out.reshape(q.shape)
```
